```python
import os as _os
_os.environ.setdefault('JAX_PLATFORMS', 'cpu')
import jax
import jax.numpy as jnp

def _softmax(x, axis=-1):
    return jax.nn.softmax(x, axis=axis)

def _gelu(x):
    return jax.nn.gelu(x, approximate=True)

def _silu(x):
    return jax.nn.silu(x)

def _sigmoid(x):
    return jax.nn.sigmoid(x)

def _layernorm(x, axis=-1, eps=1e-05):
    m = jnp.mean(x, axis=axis, keepdims=True)
    v = jnp.var(x, axis=axis, keepdims=True)
    return (x - m) / jnp.sqrt(v + eps)

def _scatter_add(tgt, idx, src, axis=0):
    return tgt.at[idx].add(src)

def _segment_sum(src, seg, n):
    return jax.ops.segment_sum(src, seg, n)

class _Rng:

    def __init__(self, key):
        self._k = key

    def _next(self):
        self._k, sub = jax.random.split(self._k)
        return sub

    def normal(self, shape):
        return jax.random.normal(self._next(), shape, dtype=jnp.bfloat16)

    def randint(self, lo, hi, shape):
        return jax.random.randint(self._next(), shape, lo, hi, dtype=jnp.int32)

    def uniform(self, shape, lo=0.0, hi=1.0):
        return jax.random.uniform(self._next(), shape, jnp.bfloat16, lo, hi)

    def permutation(self, n):
        return jax.random.permutation(self._next(), n)
kernel_name = 'parallel_sum__memory_aug_recurrent_mem_tr__dense_activation_gelu__prompt'

def setup_inputs():
    _rng = _Rng(jax.random.key(int.from_bytes(__import__("os").urandom(4), "little")))
    _w = lambda a: (lambda t: t.astype(jnp.bfloat16) if jnp.issubdtype(t.dtype, jnp.floating) else t)(jnp.asarray(a))

    def _A_setup():
        B, S, Dm = (1, 2048, 1024)
        H, Dh = (32, 128)
        M, seg = (8, 32)
        seg = min(seg, S)
        S = S // seg * seg
        return {'x': _w((lambda *s: _rng.normal(s) * 0.05)(B, S, Dm)), 'mem0': _w((lambda *s: _rng.normal(s) * 0.2)(B, M, Dm)), 'Wq': _w((lambda *s: _rng.normal(s) * 0.8)(Dm, H, Dh) * Dm ** (-0.5)), 'Wk': _w((lambda *s: _rng.normal(s) * 0.8)(Dm, H, Dh) * Dm ** (-0.5)), 'Wv': _w((lambda *s: _rng.normal(s) * 0.2)(Dm, H, Dh) * Dm ** (-0.5)), 'Wo': _w((lambda *s: _rng.normal(s) * 0.2)(H, Dh, Dm) * (H * Dh) ** (-0.5)), 'seg_len': seg}
    _A_in = _A_setup()

    def _B_setup():
        B, S, D, F = (1, 2048, 1024, 3584)
        return {'x': _w((lambda *s: _rng.normal(s) * 0.05)(B, S, D)), 'w1': _w((lambda *s: _rng.normal(s) * 0.1)(D, F) * D ** (-0.5)), 'b1': _w((lambda *s: _rng.normal(s) * 0.1)(F) * 0.01), 'w2': _w((lambda *s: _rng.normal(s) * 0.1)(F, D) * F ** (-0.5)), 'b2': _w((lambda *s: _rng.normal(s) * 0.05)(D) * 0.01)}
    _B_in = _B_setup()
    return {'A_x': _A_in['x'], 'A_mem0': _A_in['mem0'], 'A_Wq': _A_in['Wq'], 'A_Wk': _A_in['Wk'], 'A_Wv': _A_in['Wv'], 'A_Wo': _A_in['Wo'], 'A_seg_len': _A_in['seg_len'], 'B_x': _B_in['x'], 'B_w1': _B_in['w1'], 'B_b1': _B_in['b1'], 'B_w2': _B_in['w2'], 'B_b2': _B_in['b2']}

def reference(A_x, A_mem0, A_Wq, A_Wk, A_Wv, A_Wo, A_seg_len, B_x, B_w1, B_b1, B_w2, B_b2):

    def _A_ref(x, mem0, Wq, Wk, Wv, Wo, seg_len):
        B, S, Dm = x.shape
        H, Dh = (Wq.shape[1], Wq.shape[2])
        M = mem0.shape[1]
        scale = Dh ** (-0.5)
        n_seg = S // seg_len
        L = M + seg_len
        idx = jnp.arange(L)
        mask = (idx[:, None] < M) | (idx[:, None] >= idx[None, :])
        mem = mem0
        outs = []
        for s in range(n_seg):
            xs = x[:, s * seg_len:(s + 1) * seg_len, :].copy()
            h = jnp.concatenate([mem, xs], axis=1)
            q = jnp.einsum('btd,dhe->bhte', h, Wq)
            k = jnp.einsum('btd,dhe->bhte', h, Wk)
            v = jnp.einsum('btd,dhe->bhte', h, Wv)
            scores = jnp.einsum('bhqe,bhke->bhqk', q, k) * scale
            scores = jnp.where(mask[None, None], scores, -1000000000.0)
            p = _softmax(scores, axis=-1)
            o = jnp.einsum('bhqk,bhke->bhqe', p, v)
            o = jnp.einsum('bhte,hed->btd', o, Wo)
            mem = o[:, :M, :].copy()
            outs.append(o[:, M:, :])
        return jnp.concatenate(outs, axis=1)

    def _B_ref(x, w1, b1, w2, b2):
        h = jnp.einsum('bsd,df->bsf', x, w1) + b1
        h = _gelu(h)
        return jnp.einsum('bsf,fd->bsd', h, w2) + b2
    x = A_x
    xn = _layernorm(x, axis=-1)
    return x + _A_ref(xn, A_mem0, A_Wq, A_Wk, A_Wv, A_Wo, A_seg_len) + _B_ref(xn, B_w1, B_b1, B_w2, B_b2)
```

```python
import functools

import jax
import jax.numpy as jnp
from jax import lax
import jax.experimental.pallas as pl
import jax.experimental.pallas.tpu as pltpu

_F32 = jnp.float32
_BF16 = jnp.bfloat16
_LANE = 128

_CH3 = 64
_PR = 16
_KC = 4
_LAG = 4
_WO_AT = 24
_HEAD_GROUPS = 4


def _make_kernel(seg, M, H, Dh, D, F, G, NG):
    A = seg - M
    L = seg + M
    scale = Dh ** -0.5
    HD = H * Dh
    rows = seg * G
    nq = HD // _LANE
    nd = D // _LANE
    nf = F // _LANE
    hpg = H // _HEAD_GROUPS
    NCH = D // _CH3
    CPI = 3 * NCH // NG

    def wtile(w_u, j, k0=None, k1=None):
        if k0 is None:
            blk = w_u[:, j * _LANE:(j + 1) * _LANE]
        else:
            blk = w_u[k0 // 2:k1 // 2, j * _LANE:(j + 1) * _LANE]
        return pltpu.bitcast(blk, _BF16)

    def mm(lhs, w_u, panels):
        return jnp.concatenate(
            [jnp.dot(lhs, wtile(w_u, j), preferred_element_type=_F32) for j in panels], axis=1)

    def kernel(mem0_ref, b1_ref, b2_ref, x_hbm, wq_hbm, wk_hbm, wv_hbm, wo_hbm, w1_hbm, w2_hbm,
               o_ref,
               wqkv_p, wo_p, w1_s, w2_s, xn_all, base_all, x_st, st_a, st_b, hm_ref,
               mem_ref, qkvB_ref, attB_ref, acc_ref, sem_x, sem3, sem_w):
        step = pl.program_id(0)
        w3 = (wq_hbm, wk_hbm, wv_hbm)

        def cpx(g, slot):
            return pltpu.make_async_copy(x_hbm.at[pl.ds(g * rows, rows), :], x_st.at[slot],
                                         sem_x.at[slot])

        def cp3(m, i, sset, k):
            return pltpu.make_async_copy(w3[m].at[pl.ds(i * _CH3, _CH3)], st_a.at[sset, k],
                                         sem3.at[sset * CPI + k])

        def wait3(sset, k):
            pltpu.make_async_copy(st_a.at[sset, k], st_a.at[sset, k],
                                  sem3.at[sset * CPI + k]).wait()

        def start3(g, sset):
            for k in range(CPI):
                c = g * CPI + k
                for m in range(3):
                    @pl.when(c // NCH == m)
                    def _():
                        cp3(m, c - m * NCH, sset, k).start()

        def cw1():
            return pltpu.make_async_copy(w1_hbm, w1_s, sem_w.at[0])

        def cw2():
            return pltpu.make_async_copy(w2_hbm, w2_s, sem_w.at[1])

        def cwo():
            return pltpu.make_async_copy(wo_hbm, st_b, sem_w.at[2])

        @pl.when(step == 0)
        def _():
            cpx(0, 0).start()
            cw1().start()
            cw2().start()
            for k in range(CPI):
                cp3(k // NCH, k % NCH, 0, k).start()

            def ffn_iter(g, carry):
                slot = g % 2
                cpx(g, slot).wait()

                @pl.when(g == 0)
                def _():
                    cw1().wait()
                    cw2().wait()

                for k in range(CPI):
                    wait3(slot, k)

                @pl.when(g + 1 < NG)
                def _():
                    cpx(g + 1, 1 - slot).start()
                    start3(g + 1, 1 - slot)

                @pl.when(g == NG // 2)
                def _():
                    cwo().start()

                r0 = pl.multiple_of(g * rows, rows)
                x = x_st[slot].astype(_F32)
                mu = jnp.mean(x, axis=-1, keepdims=True)
                xc = x - mu
                var = jnp.mean(xc * xc, axis=-1, keepdims=True)
                xn = (xc * lax.rsqrt(var + 1e-5)).astype(_BF16)
                xn_all[pl.ds(r0, rows), :] = xn.astype(_F32)

                pieces = [(k, pc) for k in range(CPI) for pc in range(_CH3 // _PR)]

                def relayout_piece(k, pc):
                    c = g * CPI + k
                    q0 = pl.multiple_of((c % NCH) * (_CH3 // 2) + pc * (_PR // 2), 8)
                    col0 = (c // NCH) * HD
                    u = pltpu.bitcast(st_a[slot, k, pc * _PR:(pc + 1) * _PR], jnp.uint32)
                    u4 = u.reshape(_PR // 2, 2, H // 2, Dh)
                    a, b = u4[:, 0], u4[:, 1]
                    lo = jnp.swapaxes((a & jnp.uint32(0xffff)) | (b << 16), 0, 1)
                    hi = jnp.swapaxes((a >> 16) | (b & jnp.uint32(0xffff0000)), 0, 1)
                    for hp in range(H // 2):
                        c_lo = pl.multiple_of(col0 + 2 * hp * Dh, Dh)
                        c_hi = pl.multiple_of(col0 + (2 * hp + 1) * Dh, Dh)
                        wqkv_p[pl.ds(q0, _PR // 2), pl.ds(c_lo, Dh)] = lo[hp]
                        wqkv_p[pl.ds(q0, _PR // 2), pl.ds(c_hi, Dh)] = hi[hp]

                kc = F // _KC
                every = max(1, (nf + nd * _KC) // len(pieces))
                ticks = [0]

                def tick():
                    ticks[0] += 1
                    if ticks[0] % every == 0 and pieces:
                        relayout_piece(*pieces.pop(0))

                for j in range(nf):
                    hm = (jnp.dot(xn, w1_s[:, j * _LANE:(j + 1) * _LANE],
                                  preferred_element_type=_F32)
                          + b1_ref[:, j * _LANE:(j + 1) * _LANE].astype(_F32))
                    hm_ref[:, j * _LANE:(j + 1) * _LANE] = (
                        jax.nn.gelu(hm, approximate=True).astype(_BF16))
                    tick()
                for j in range(nd):
                    acc = (x[:, j * _LANE:(j + 1) * _LANE]
                           + b2_ref[:, j * _LANE:(j + 1) * _LANE].astype(_F32))
                    for q in range(_KC):
                        acc = acc + jnp.dot(hm_ref[:, q * kc:(q + 1) * kc],
                                            w2_s[q * kc:(q + 1) * kc, j * _LANE:(j + 1) * _LANE],
                                            preferred_element_type=_F32)
                        tick()
                    base_all[pl.ds(r0, rows), j * _LANE:(j + 1) * _LANE] = acc
                while pieces:
                    relayout_piece(*pieces.pop(0))
                return carry

            lax.fori_loop(0, NG, ffn_iter, 0)
            cwo().wait()
            n = HD // 8
            for i in range(8):
                wo_p[i * (n // 2):(i + 1) * (n // 2), :] = pltpu.bitcast(
                    st_b[i * n:(i + 1) * n, :], jnp.uint32)
            mem_ref[...] = mem0_ref[...].astype(_F32)

        g0 = pl.multiple_of(step * rows, rows)

        hB = jnp.concatenate([xn_all[pl.ds(g0 + s * seg + A, M), :] for s in range(G)],
                             axis=0).astype(_BF16)
        qkvB_ref[...] = mm(hB, wqkv_p, range(3 * nq))

        r = lax.broadcasted_iota(jnp.int32, (L, L), 0)
        c = lax.broadcasted_iota(jnp.int32, (L, L), 1)
        is_mem_r = (r >= A) & (r < seg)
        is_mem_c = (c >= A) & (c < seg)
        xpos_r = jnp.where(r < A, r, r - M)
        xpos_c = jnp.where(c < A, c, c - M)
        mask = is_mem_r | is_mem_c | (xpos_c <= xpos_r)

        def seg_body(s, mem):
            row0 = pl.multiple_of(s * seg, seg)
            brow = pl.multiple_of(s * M, M)
            hA = jnp.concatenate([xn_all[pl.ds(pl.multiple_of(g0 + row0, seg), A), :], mem],
                                 axis=0).astype(_BF16)

            def qkv_head(hd):
                res = []
                for m in range(3):
                    pa = jnp.dot(hA, wtile(wqkv_p, m * nq + hd), preferred_element_type=_F32)
                    pb = qkvB_ref[pl.ds(brow, M), (m * H + hd) * Dh:(m * H + hd + 1) * Dh]
                    res.append(jnp.concatenate([pa, pb], axis=0).astype(_BF16))
                return res

            def attn(q, k, v):
                sc = lax.dot_general(q, k, (((1,), (1,)), ((), ())),
                                     preferred_element_type=_F32) * scale
                sc = jnp.where(mask, sc, -1e9)
                mx = jnp.max(sc, axis=-1, keepdims=True)
                p = jnp.exp(sc - mx)
                p = p / jnp.sum(p, axis=-1, keepdims=True)
                o = jnp.dot(p.astype(_BF16), v, preferred_element_type=_F32)
                return o.astype(_BF16).astype(_F32)

            qkv = {hd: qkv_head(hd) for hd in range(_LAG)}
            o_acc = [None] * nd
            grp, done, pending = [], [], []

            def wo_panel(g, j):
                part = jnp.dot(done[g], wtile(wo_p, j, g * hpg * Dh, (g + 1) * hpg * Dh),
                               preferred_element_type=_F32)
                o_acc[j] = part if o_acc[j] is None else o_acc[j] + part

            for hd in range(H):
                if hd + _LAG < H:
                    qkv[hd + _LAG] = qkv_head(hd + _LAG)
                a = attn(*qkv.pop(hd))
                attB_ref[pl.ds(brow, M), hd * Dh:(hd + 1) * Dh] = a[seg:]
                grp.append(a[:seg].astype(_BF16))
                if len(grp) == hpg:
                    done.append(jnp.concatenate(grp, axis=1))
                    pending += [(len(done) - 1, j) for j in range(nd)]
                    grp = []
                if hd >= _WO_AT:
                    n_issue = -(-len(pending) // (H - hd)) if hd < H - 1 else len(pending)
                    for (g, j) in pending[:n_issue]:
                        wo_panel(g, j)
                    pending = pending[n_issue:]
            o = jnp.concatenate(o_acc, axis=1)
            acc_ref[pl.ds(row0, A), :] = o[:A]
            return o[A:seg].astype(_BF16).astype(_F32)

        mem = lax.fori_loop(0, G, seg_body, mem_ref[...])
        mem_ref[...] = mem

        oB = mm(attB_ref[...].astype(_BF16), wo_p, range(nd))
        for s in range(G):
            acc_ref[s * seg + A:(s + 1) * seg, :] = oB[s * M:(s + 1) * M]
        o_ref[...] = (base_all[pl.ds(g0, rows), :] + acc_ref[...]).astype(o_ref.dtype)

    return kernel, CPI


@functools.partial(jax.jit, static_argnames=("A_seg_len",))
def pallas_parallel_sum__memory_aug_recurrent_mem_tr__dense_activation_gelu__prompt_kernel(
    A_x: jax.Array,
    A_mem0: jax.Array,
    A_Wq: jax.Array,
    A_Wk: jax.Array,
    A_Wv: jax.Array,
    A_Wo: jax.Array,
    A_seg_len,
    B_x: jax.Array,
    B_w1: jax.Array,
    B_b1: jax.Array,
    B_w2: jax.Array,
    B_b2: jax.Array,
):
    del B_x
    B, S, D = A_x.shape
    H, Dh = A_Wq.shape[1], A_Wq.shape[2]
    M = A_mem0.shape[1]
    F = B_w1.shape[1]
    seg = int(A_seg_len)
    HD = H * Dh
    G = seg // M
    rows = seg * G
    NG = S // rows
    assert B == 1 and seg % M == 0 and S % rows == 0 and Dh == _LANE
    assert D % _CH3 == 0 and (3 * (D // _CH3)) % NG == 0 and F % (_KC * _LANE) == 0
    assert H % (2 * _HEAD_GROUPS) == 0 and HD % 16 == 0

    x2 = A_x.reshape(S, D)
    mem0 = A_mem0.reshape(M, D)
    wo = A_Wo.reshape(HD, D)
    b1 = B_b1.reshape(1, F)
    b2 = B_b2.reshape(1, D)

    kernel, cpi = _make_kernel(seg, M, H, Dh, D, F, G, NG)
    const = lambda shape: pl.BlockSpec(shape, lambda i: (0,) * len(shape))
    hbm = pl.BlockSpec(memory_space=pl.ANY)

    out = pl.pallas_call(
        kernel,
        grid=(NG,),
        in_specs=[const((M, D)), const((1, F)), const((1, D)),
                  hbm, hbm, hbm, hbm, hbm, hbm, hbm],
        out_specs=pl.BlockSpec((rows, D), lambda i: (i, 0)),
        out_shape=jax.ShapeDtypeStruct((S, D), A_x.dtype),
        scratch_shapes=[
            pltpu.VMEM((D // 2, 3 * HD), jnp.uint32),
            pltpu.VMEM((HD // 2, D), jnp.uint32),
            pltpu.VMEM((D, F), _BF16),
            pltpu.VMEM((F, D), _BF16),
            pltpu.VMEM((S, D), _F32),
            pltpu.VMEM((S, D), _F32),
            pltpu.VMEM((2, rows, D), _BF16),
            pltpu.VMEM((2, cpi, _CH3, H, Dh), _BF16),
            pltpu.VMEM((HD, D), _BF16),
            pltpu.VMEM((rows, F), _BF16),
            pltpu.VMEM((M, D), _F32),
            pltpu.VMEM((G * M, 3 * HD), _F32),
            pltpu.VMEM((G * M, HD), _F32),
            pltpu.VMEM((rows, D), _F32),
            pltpu.SemaphoreType.DMA((2,)),
            pltpu.SemaphoreType.DMA((2 * cpi,)),
            pltpu.SemaphoreType.DMA((3,)),
        ],
        compiler_params=pltpu.CompilerParams(
            dimension_semantics=("arbitrary",),
            vmem_limit_bytes=110 * 1024 * 1024),
    )(mem0, b1, b2, x2, A_Wq, A_Wk, A_Wv, wo, B_w1, B_w2)
    return out.reshape(B, S, D)
```
